```python
import os as _os
_os.environ.setdefault("JAX_PLATFORMS", "cpu")
import jax
import jax.numpy as jnp

def _softmax(x, axis=-1):
    return jax.nn.softmax(x, axis=axis)
def _gelu(x):
    return jax.nn.gelu(x, approximate=True)
def _silu(x):
    return jax.nn.silu(x)
def _sigmoid(x):
    return jax.nn.sigmoid(x)
def _layernorm(x, axis=-1, eps=1e-5):
    m = jnp.mean(x, axis=axis, keepdims=True)
    v = jnp.var(x, axis=axis, keepdims=True)
    return (x - m) / jnp.sqrt(v + eps)
def _scatter_add(tgt, idx, src, axis=0):
    return tgt.at[idx].add(src)
def _segment_sum(src, seg, n):
    return jax.ops.segment_sum(src, seg, n)
class _Rng:
    def __init__(self, key):
        self._k = key
    def _next(self):
        self._k, sub = jax.random.split(self._k)
        return sub
    def normal(self, shape):
        return jax.random.normal(self._next(), shape, dtype=jnp.bfloat16)
    def randint(self, lo, hi, shape):
        return jax.random.randint(self._next(), shape, lo, hi, dtype=jnp.int32)
    def uniform(self, shape, lo=0.0, hi=1.0):
        return jax.random.uniform(self._next(), shape, jnp.bfloat16, lo, hi)
    def permutation(self, n):
        return jax.random.permutation(self._next(), n)


kernel_name = 'sequential_preLN__ssm_conv_h3__mixer_s_mlp__prompt'

def setup_inputs():
    _rng = _Rng(jax.random.key(int.from_bytes(__import__("os").urandom(4), "little")))
    _w = (lambda a: (lambda t: t.astype(jnp.bfloat16) if jnp.issubdtype(t.dtype, jnp.floating) else t)(jnp.asarray(a)))
    def _A_setup():
        B, S, D = 1, 2048, 640
        ks = 4
        return {
            "q": _w((lambda *s: _rng.normal(s) * 0.05)(B, S, D)),
            "k": _w((lambda *s: _rng.normal(s) * 0.05)(B, S, D)),
            "v": _w((lambda *s: _rng.normal(s) * 0.05)(B, S, D)),
            "shift_k": _w((lambda *s: _rng.normal(s) * 0.05)(D, ks) * 0.5),
            "ssm_k": _w((lambda *s: _rng.normal(s) * 0.05)(D, S) * (1.0 / S ** 0.5)),
            "ssm_D": _w((lambda *s: _rng.normal(s) * 0.05)(D)),
        }
    _A_in = _A_setup()

    def _B_setup():
        B, S, D, F = 1, 2048, 640, 1728
        return {
            "x":  _w((lambda *s: _rng.normal(s) * 0.05)(B, S, D)),
            "w1": _w((lambda *s: _rng.normal(s) * 0.8)(D, D) * (D ** -0.5)),
            "w2": _w((lambda *s: _rng.normal(s) * 0.8)(D, D) * (D ** -0.5)),
            "w3": _w((lambda *s: _rng.normal(s) * 0.8)(D, F) * (D ** -0.5)),
            "w4": _w((lambda *s: _rng.normal(s) * 0.8)(F, D) * (F ** -0.5)),
        }
    _B_in = _B_setup()

    return {
        "A_q": _A_in["q"],
        "A_k": _A_in["k"],
        "A_v": _A_in["v"],
        "A_shift_k": _A_in["shift_k"],
        "A_ssm_k": _A_in["ssm_k"],
        "A_ssm_D": _A_in["ssm_D"],
        "B_x": _B_in["x"],
        "B_w1": _B_in["w1"],
        "B_w2": _B_in["w2"],
        "B_w3": _B_in["w3"],
        "B_w4": _B_in["w4"],
    }

def reference(A_q, A_k, A_v, A_shift_k, A_ssm_k, A_ssm_D, B_x, B_w1, B_w2, B_w3, B_w4):
    def _A_ref(q, k, v, shift_k, ssm_k, ssm_D):
        B, S, D = q.shape
        ks = shift_k.shape[-1]
        k_pad = jnp.pad(k, ((0, 0), (ks - 1, 0), (0, 0)))
        k_shift = jnp.zeros_like(k)
        for t in range(ks):
            k_shift = k_shift + k_pad[:, t:t + S, :] * shift_k[:, ks - 1 - t][None, None, :]
        kv = k_shift * v
        L = 2 * S
        kv_pad = jnp.pad(kv, ((0, 0), (0, S), (0, 0)))
        kf_pad = jnp.pad(ssm_k, ((0, 0), (0, S)))
        kv_f = (lambda x, axes=(-2,-1): jnp.fft.rfft2(x.astype(jnp.float32), axes=axes))(kv_pad[:, None, :, :], axes=(1, 2))
        kf_f = (lambda x, axes=(-2,-1): jnp.fft.rfft2(x.astype(jnp.float32), axes=axes))(kf_pad[:, None, :], axes=(1, 2))
        kf_f = (lambda x, *d: x.transpose(*d))(kf_f, 1, 2, 0)
        y_f = kv_f * kf_f[None, :, :, :]
        y = (lambda x, s, axes=(-2,-1): jnp.fft.irfft2(x, s=s, axes=axes).astype(jnp.bfloat16))(y_f, (1, L), axes=(1, 2))[:, 0, :S, :]
        y = y + kv * ssm_D[None, None, :]
        return q * y

    def _B_ref(x, w1, w2, w3, w4):
        B, S, D = x.shape
        h = _gelu(_layernorm(x, axis=-1) @ w1)
        c = D // 4
        g0 = jnp.pad(h[:, :, 0*c:1*c], ((0, 0), (1, 0), (0, 0)))[:, :S, :]
        g1 = jnp.pad(h[:, :, 1*c:2*c], ((0, 0), (0, 1), (0, 0)))[:, 1:, :]
        g2 = jnp.pad(h[:, :, 2*c:3*c], ((0, 0), (2, 0), (0, 0)))[:, :S, :]
        g3 = jnp.pad(h[:, :, 3*c:   ], ((0, 0), (0, 2), (0, 0)))[:, 2:, :]
        hs = jnp.concatenate([g0, g1, g2, g3], axis=-1) @ w2
        x1 = x + hs
        h2 = _gelu(_layernorm(x1, axis=-1) @ w3) @ w4
        return x1 + h2

    x = A_q
    h = x + _A_ref(_layernorm(x, axis=-1), A_k, A_v, A_shift_k, A_ssm_k, A_ssm_D)
    h2 = h + _B_ref(_layernorm(h, axis=-1), B_w1, B_w2, B_w3, B_w4)
    return h2
```

```python
import numpy as np
import jax
import jax.numpy as jnp
import jax.experimental.pallas as pl
import jax.experimental.pallas.tpu as pltpu

_BLK = 256
_EPS = 1e-5
_PAD = 8


def _dft_tables(n2):
    n = np.arange(n2)
    w = np.arange(n2)
    ph = ((2 * w[:, None] + 1) * n[None, :]) % (4 * n2)
    th = 2.0 * np.pi * ph.astype(np.float64) / (4 * n2)
    ff = np.concatenate([np.cos(th), -np.sin(th)], axis=0)
    gi = np.concatenate([np.cos(th).T, -np.sin(th).T], axis=1) / n2
    sgn = ((-1.0) ** w)[:, None]
    return ff, gi, sgn


def _ln(x):
    m = jnp.mean(x, axis=-1, keepdims=True)
    xc = x - m
    v = jnp.mean(xc * xc, axis=-1, keepdims=True)
    return xc * jax.lax.rsqrt(v + _EPS)


def _gelu(x):
    return jax.nn.gelu(x, approximate=True)


def _make_kernel(S, D, F, NB, KS):
    BLK = _BLK
    C = D // 4

    def kernel(q_ref, k_ref, v_ref, sk_ref, ssmk_ref, ssmd_ref,
               w1_ref, w2_ref, w3_ref, w4_ref, ff_ref, gi_ref, sgn_ref,
               o_ref,
               u_scr, kp_scr, kraw_scr, kext_scr, h_scr, xb_scr, h1_scr, z_scr):
        c = pl.program_id(0)

        @pl.when(c == 0)
        def _init():
            kext_scr[...] = jnp.zeros(kext_scr.shape, jnp.float32)
            kraw_scr[...] = jnp.zeros(kraw_scr.shape, jnp.float32)
            h1_scr[pl.ds(0, _PAD), :] = jnp.zeros((_PAD, D), jnp.float32)
            h1_scr[pl.ds(S + _PAD, _PAD), :] = jnp.zeros((_PAD, D), jnp.float32)

        @pl.when(c < NB)
        def _phase_a():
            kext_scr[pl.ds(0, _PAD), :] = kext_scr[pl.ds(BLK, _PAD), :]
            kext_scr[pl.ds(_PAD, BLK), :] = k_ref[...].astype(jnp.float32)
            ks = jnp.zeros((BLK, D), jnp.float32)
            for j in range(KS):
                ks = ks + kext_scr[pl.ds(_PAD - j, BLK), :] * sk_ref[pl.ds(j, 1), :].astype(jnp.float32)
            kv = ks * v_ref[...].astype(jnp.float32)
            kv_b = kv.astype(jnp.bfloat16)

            ff = ff_ref[...]
            u_scr[c] = jnp.dot(ff, kv_b, preferred_element_type=jnp.float32)
            kraw = jax.lax.dot_general(
                ff, ssmk_ref[...], (((1,), (1,)), ((), ())),
                preferred_element_type=jnp.float32)
            sgn = sgn_ref[...]
            prev = kraw_scr[...]
            kp_scr[c, pl.ds(0, BLK), :] = kraw[:BLK] - sgn * prev[BLK:]
            kp_scr[c, pl.ds(BLK, BLK), :] = kraw[BLK:] + sgn * prev[:BLK]
            kraw_scr[...] = kraw

            z_scr[...] = jnp.zeros(z_scr.shape, jnp.float32)

            def body(j, carry):
                kr = kp_scr[j, pl.ds(0, BLK), :]
                ki = kp_scr[j, pl.ds(BLK, BLK), :]
                ur = u_scr[c - j, pl.ds(0, BLK), :]
                ui = u_scr[c - j, pl.ds(BLK, BLK), :]
                z_scr[pl.ds(0, BLK), :] += kr * ur - ki * ui
                z_scr[pl.ds(BLK, BLK), :] += kr * ui + ki * ur
                return carry

            jax.lax.fori_loop(0, c + 1, body, 0)
            y = jnp.dot(gi_ref[...], z_scr[...].astype(jnp.bfloat16),
                        preferred_element_type=jnp.float32)
            y = y + kv * ssmd_ref[...].astype(jnp.float32)

            x = q_ref[...].astype(jnp.float32)
            h = x + _ln(x) * y
            xb = _ln(h)
            row0 = pl.multiple_of(c * BLK, BLK)
            h_scr[pl.ds(row0, BLK), :] = h
            xb_scr[pl.ds(row0, BLK), :] = xb
            h1 = _gelu(jnp.dot(_ln(xb).astype(jnp.bfloat16), w1_ref[...],
                               preferred_element_type=jnp.float32))
            h1_scr[pl.ds(row0 + _PAD, BLK), :] = h1

        @pl.when(c >= 1)
        def _phase_b():
            b = c - 1
            row0 = pl.multiple_of(b * BLK, BLK)
            col = jax.lax.broadcasted_iota(jnp.int32, (BLK, D), 1)
            win = h1_scr[pl.ds(row0, BLK + 2 * _PAD), :]
            g0 = win[_PAD - 1:_PAD - 1 + BLK]
            g1 = win[_PAD + 1:_PAD + 1 + BLK]
            g2 = win[_PAD - 2:_PAD - 2 + BLK]
            g3 = win[_PAD + 2:_PAD + 2 + BLK]
            hs_in = jnp.where(col < C, g0,
                              jnp.where(col < 2 * C, g1,
                                        jnp.where(col < 3 * C, g2, g3)))
            hs = jnp.dot(hs_in.astype(jnp.bfloat16), w2_ref[...],
                         preferred_element_type=jnp.float32)
            x1 = xb_scr[pl.ds(row0, BLK), :] + hs
            t = _gelu(jnp.dot(_ln(x1).astype(jnp.bfloat16), w3_ref[...],
                              preferred_element_type=jnp.float32))
            h2 = jnp.dot(t.astype(jnp.bfloat16), w4_ref[...],
                         preferred_element_type=jnp.float32)
            o_ref[...] = (h_scr[pl.ds(row0, BLK), :] + x1 + h2).astype(o_ref.dtype)

    return kernel


@jax.jit
def pallas_sequential_preLN__ssm_conv_h3__mixer_s_mlp__prompt_kernel(
    A_q: jax.Array,
    A_k: jax.Array,
    A_v: jax.Array,
    A_shift_k: jax.Array,
    A_ssm_k: jax.Array,
    A_ssm_D: jax.Array,
    B_x: jax.Array,
    B_w1: jax.Array,
    B_w2: jax.Array,
    B_w3: jax.Array,
    B_w4: jax.Array,
):
    Bsz, S, D = A_q.shape
    assert Bsz == 1
    F = B_w3.shape[1]
    KS = A_shift_k.shape[1]
    BLK = _BLK
    NB = S // BLK
    assert S % BLK == 0

    q = A_q.reshape(S, D)
    k = A_k.reshape(S, D)
    v = A_v.reshape(S, D)
    sk = A_shift_k.T
    ssmd = A_ssm_D.reshape(1, D)

    ff_np, gi_np, sgn_np = _dft_tables(BLK)
    ff = jnp.asarray(ff_np, dtype=jnp.bfloat16)
    gi = jnp.asarray(gi_np, dtype=jnp.bfloat16)
    sgn = jnp.asarray(sgn_np, dtype=jnp.float32)

    row_in = lambda c: (jnp.minimum(c, NB - 1), 0)
    full = lambda c: (0, 0)

    kernel = _make_kernel(S, D, F, NB, KS)
    out = pl.pallas_call(
        kernel,
        grid=(NB + 1,),
        in_specs=[
            pl.BlockSpec((BLK, D), row_in),
            pl.BlockSpec((BLK, D), row_in),
            pl.BlockSpec((BLK, D), row_in),
            pl.BlockSpec((KS, D), full),
            pl.BlockSpec((D, BLK), lambda c: (0, jnp.minimum(c, NB - 1))),
            pl.BlockSpec((1, D), full),
            pl.BlockSpec((D, D), full),
            pl.BlockSpec((D, D), full),
            pl.BlockSpec((D, F), full),
            pl.BlockSpec((F, D), full),
            pl.BlockSpec((2 * BLK, BLK), full),
            pl.BlockSpec((BLK, 2 * BLK), full),
            pl.BlockSpec((BLK, 1), full),
        ],
        out_specs=pl.BlockSpec((BLK, D), lambda c: (jnp.maximum(c - 1, 0), 0)),
        out_shape=jax.ShapeDtypeStruct((S, D), A_q.dtype),
        scratch_shapes=[
            pltpu.VMEM((NB, 2 * BLK, D), jnp.float32),
            pltpu.VMEM((NB, 2 * BLK, D), jnp.float32),
            pltpu.VMEM((2 * BLK, D), jnp.float32),
            pltpu.VMEM((BLK + _PAD, D), jnp.float32),
            pltpu.VMEM((S, D), jnp.float32),
            pltpu.VMEM((S, D), jnp.float32),
            pltpu.VMEM((S + 2 * _PAD, D), jnp.float32),
            pltpu.VMEM((2 * BLK, D), jnp.float32),
        ],
        compiler_params=pltpu.CompilerParams(
            dimension_semantics=("arbitrary",),
            vmem_limit_bytes=100 * 1024 * 1024,
        ),
    )(q, k, v, sk, A_ssm_k, ssmd, B_w1, B_w2, B_w3, B_w4, ff, gi, sgn)
    return out.reshape(Bsz, S, D)
```

```python
import numpy as np
import jax
import jax.numpy as jnp
import jax.experimental.pallas as pl
import jax.experimental.pallas.tpu as pltpu

_BLK = 256
_EPS = 1e-5
_PAD = 8


def _dft_tables(n2):
    n = np.arange(n2)
    w = np.arange(n2)
    ph = ((2 * w[:, None] + 1) * n[None, :]) % (4 * n2)
    th = 2.0 * np.pi * ph.astype(np.float64) / (4 * n2)
    ff = np.concatenate([np.cos(th), -np.sin(th)], axis=0)
    gi = np.concatenate([np.cos(th).T, -np.sin(th).T], axis=1) / n2
    sgn = ((-1.0) ** w)[:, None]
    return ff, gi, sgn


def _ln(x):
    m = jnp.mean(x, axis=-1, keepdims=True)
    xc = x - m
    v = jnp.mean(xc * xc, axis=-1, keepdims=True)
    return xc * jax.lax.rsqrt(v + _EPS)


def _gelu(x):
    return jax.nn.gelu(x, approximate=True)


def _make_kernel(S, D, F, NB, KS):
    BLK = _BLK
    C = D // 4
    LAG = 2

    def kernel(q_ref, k_ref, v_ref, sk_ref, ssmk_ref, ssmd_ref,
               w1_hbm, w2_hbm, w3t_hbm, w4_hbm, ff_ref, gi_ref, sgn_ref,
               o_ref,
               u_scr, kp_scr, kraw_scr, kext_scr, h_scr, xb_scr, h1_scr,
               z_scr, w1_ref, w2_ref, w3t_ref, w4_ref, sems):
        c = pl.program_id(0)

        w_copies = [
            pltpu.make_async_copy(w1_hbm, w1_ref, sems.at[0]),
            pltpu.make_async_copy(w2_hbm, w2_ref, sems.at[1]),
            pltpu.make_async_copy(w3t_hbm, w3t_ref, sems.at[2]),
            pltpu.make_async_copy(w4_hbm, w4_ref, sems.at[3]),
        ]

        def phase_a(cc):
            kext_scr[pl.ds(0, _PAD), :] = kext_scr[pl.ds(BLK, _PAD), :]
            kext_scr[pl.ds(_PAD, BLK), :] = k_ref[...].astype(jnp.float32)
            ks = jnp.zeros((BLK, D), jnp.float32)
            for j in range(KS):
                ks = ks + kext_scr[pl.ds(_PAD - j, BLK), :] * sk_ref[pl.ds(j, 1), :].astype(jnp.float32)
            kv = ks * v_ref[...].astype(jnp.float32)
            kv_b = kv.astype(jnp.bfloat16)

            ff = ff_ref[...]
            u_scr[cc] = jnp.dot(ff, kv_b, preferred_element_type=jnp.float32)
            kraw = jax.lax.dot_general(
                ff, ssmk_ref[...], (((1,), (1,)), ((), ())),
                preferred_element_type=jnp.float32)
            sgn = sgn_ref[...]
            prev = kraw_scr[...]
            kp_scr[cc, pl.ds(0, BLK), :] = kraw[:BLK] - sgn * prev[BLK:]
            kp_scr[cc, pl.ds(BLK, BLK), :] = kraw[BLK:] + sgn * prev[:BLK]
            kraw_scr[...] = kraw

            z_scr[...] = jnp.zeros(z_scr.shape, jnp.float32)

            def body(j, carry):
                kr = kp_scr[j, pl.ds(0, BLK), :]
                ki = kp_scr[j, pl.ds(BLK, BLK), :]
                ur = u_scr[cc - j, pl.ds(0, BLK), :]
                ui = u_scr[cc - j, pl.ds(BLK, BLK), :]
                z_scr[pl.ds(0, BLK), :] += kr * ur - ki * ui
                z_scr[pl.ds(BLK, BLK), :] += kr * ui + ki * ur
                return carry

            jax.lax.fori_loop(0, cc + 1, body, 0)
            z = z_scr[...].astype(jnp.bfloat16)
            y = jnp.dot(gi_ref[...], z, preferred_element_type=jnp.float32)
            y = y + kv * ssmd_ref[...].astype(jnp.float32)

            x = q_ref[...].astype(jnp.float32)
            h = x + _ln(x) * y
            xb = _ln(h)
            row0 = pl.multiple_of(cc * BLK, BLK)
            h_scr[pl.ds(row0, BLK), :] = h
            xb_scr[pl.ds(row0, BLK), :] = xb
            h1 = _gelu(jnp.dot(_ln(xb).astype(jnp.bfloat16), w1_ref[...],
                               preferred_element_type=jnp.float32))
            h1_scr[pl.ds(row0 + _PAD, BLK), :] = h1

        def phase_b(b):
            row0 = pl.multiple_of(b * BLK, BLK)
            col = jax.lax.broadcasted_iota(jnp.int32, (BLK, D), 1)
            win = h1_scr[pl.ds(row0, BLK + 2 * _PAD), :]
            g0 = win[_PAD - 1:_PAD - 1 + BLK]
            g1 = win[_PAD + 1:_PAD + 1 + BLK]
            g2 = win[_PAD - 2:_PAD - 2 + BLK]
            g3 = win[_PAD + 2:_PAD + 2 + BLK]
            hs_in = jnp.where(col < C, g0,
                              jnp.where(col < 2 * C, g1,
                                        jnp.where(col < 3 * C, g2, g3)))
            hs = jnp.dot(hs_in.astype(jnp.bfloat16), w2_ref[...],
                         preferred_element_type=jnp.float32)
            x1 = xb_scr[pl.ds(row0, BLK), :] + hs
            t = _gelu(jax.lax.dot_general(
                _ln(x1).astype(jnp.bfloat16), w3t_ref[...], (((1,), (1,)), ((), ())),
                preferred_element_type=jnp.float32))
            h2 = jnp.dot(t.astype(jnp.bfloat16), w4_ref[...],
                         preferred_element_type=jnp.float32)
            o_ref[...] = (h_scr[pl.ds(row0, BLK), :] + x1 + h2).astype(o_ref.dtype)

        @pl.when(c == 0)
        def _init():
            for cp in w_copies:
                cp.start()
            kext_scr[...] = jnp.zeros(kext_scr.shape, jnp.float32)
            kraw_scr[...] = jnp.zeros(kraw_scr.shape, jnp.float32)
            h1_scr[pl.ds(0, _PAD), :] = jnp.zeros((_PAD, D), jnp.float32)
            h1_scr[pl.ds(S + _PAD, _PAD), :] = jnp.zeros((_PAD, D), jnp.float32)

        @pl.when(c == 0)
        def _wait_w1():
            w_copies[0].wait()

        @pl.when(c == LAG)
        def _wait_w():
            for cp in w_copies[1:]:
                cp.wait()

        @pl.when(c < LAG)
        def _a_only():
            phase_a(c)

        @pl.when(jnp.logical_and(c >= LAG, c < NB))
        def _ab():
            phase_b(c - LAG)
            phase_a(c)

        @pl.when(c >= NB)
        def _b_only():
            phase_b(c - LAG)

    return kernel


@jax.jit
def pallas_sequential_preLN__ssm_conv_h3__mixer_s_mlp__prompt_kernel(
    A_q: jax.Array,
    A_k: jax.Array,
    A_v: jax.Array,
    A_shift_k: jax.Array,
    A_ssm_k: jax.Array,
    A_ssm_D: jax.Array,
    B_x: jax.Array,
    B_w1: jax.Array,
    B_w2: jax.Array,
    B_w3: jax.Array,
    B_w4: jax.Array,
):
    Bsz, S, D = A_q.shape
    assert Bsz == 1
    F = B_w3.shape[1]
    KS = A_shift_k.shape[1]
    BLK = _BLK
    NB = S // BLK
    assert S % BLK == 0

    q = A_q.reshape(S, D)
    k = A_k.reshape(S, D)
    v = A_v.reshape(S, D)
    sk = A_shift_k.T
    ssmd = A_ssm_D.reshape(1, D)

    ff_np, gi_np, sgn_np = _dft_tables(BLK)
    ff = jnp.asarray(ff_np, dtype=jnp.bfloat16)
    gi = jnp.asarray(gi_np, dtype=jnp.bfloat16)
    sgn = jnp.asarray(sgn_np, dtype=jnp.float32)

    row_in = lambda c: (jnp.minimum(c, NB - 1), 0)
    full = lambda c: (0, 0)

    kernel = _make_kernel(S, D, F, NB, KS)
    out = pl.pallas_call(
        kernel,
        grid=(NB + 2,),
        in_specs=[
            pl.BlockSpec((BLK, D), row_in),
            pl.BlockSpec((BLK, D), row_in),
            pl.BlockSpec((BLK, D), row_in),
            pl.BlockSpec((KS, D), full),
            pl.BlockSpec((D, BLK), lambda c: (0, jnp.minimum(c, NB - 1))),
            pl.BlockSpec((1, D), full),
            pl.BlockSpec(memory_space=pl.ANY),
            pl.BlockSpec(memory_space=pl.ANY),
            pl.BlockSpec(memory_space=pl.ANY),
            pl.BlockSpec(memory_space=pl.ANY),
            pl.BlockSpec((2 * BLK, BLK), full),
            pl.BlockSpec((BLK, 2 * BLK), full),
            pl.BlockSpec((BLK, 1), full),
        ],
        out_specs=pl.BlockSpec((BLK, D), lambda c: (jnp.maximum(c - 2, 0), 0)),
        out_shape=jax.ShapeDtypeStruct((S, D), A_q.dtype),
        scratch_shapes=[
            pltpu.VMEM((NB, 2 * BLK, D), jnp.float32),
            pltpu.VMEM((NB, 2 * BLK, D), jnp.float32),
            pltpu.VMEM((2 * BLK, D), jnp.float32),
            pltpu.VMEM((BLK + _PAD, D), jnp.float32),
            pltpu.VMEM((S, D), jnp.float32),
            pltpu.VMEM((S, D), jnp.float32),
            pltpu.VMEM((S + 2 * _PAD, D), jnp.float32),
            pltpu.VMEM((2 * BLK, D), jnp.float32),
            pltpu.VMEM((D, D), B_w1.dtype),
            pltpu.VMEM((D, D), B_w2.dtype),
            pltpu.VMEM((F, D), B_w3.dtype),
            pltpu.VMEM((F, D), B_w4.dtype),
            pltpu.SemaphoreType.DMA((4,)),
        ],
        compiler_params=pltpu.CompilerParams(
            dimension_semantics=("arbitrary",),
            vmem_limit_bytes=100 * 1024 * 1024,
        ),
    )(q, k, v, sk, A_ssm_k, ssmd, B_w1, B_w2, B_w3.T, B_w4, ff, gi, sgn)
    return out.reshape(Bsz, S, D)
```
